```python
import os as _os
_os.environ.setdefault("JAX_PLATFORMS", "cpu")
import jax
import jax.numpy as jnp

def _softmax(x, axis=-1):
    return jax.nn.softmax(x, axis=axis)
def _gelu(x):
    return jax.nn.gelu(x, approximate=True)
def _silu(x):
    return jax.nn.silu(x)
def _sigmoid(x):
    return jax.nn.sigmoid(x)
def _layernorm(x, axis=-1, eps=1e-5):
    m = jnp.mean(x, axis=axis, keepdims=True)
    v = jnp.var(x, axis=axis, keepdims=True)
    return (x - m) / jnp.sqrt(v + eps)
def _scatter_add(tgt, idx, src, axis=0):
    return tgt.at[idx].add(src)
def _segment_sum(src, seg, n):
    return jax.ops.segment_sum(src, seg, n)
class _Rng:
    def __init__(self, key):
        self._k = key
    def _next(self):
        self._k, sub = jax.random.split(self._k)
        return sub
    def normal(self, shape):
        return jax.random.normal(self._next(), shape, dtype=jnp.bfloat16)
    def randint(self, lo, hi, shape):
        return jax.random.randint(self._next(), shape, lo, hi, dtype=jnp.int32)
    def uniform(self, shape, lo=0.0, hi=1.0):
        return jax.random.uniform(self._next(), shape, jnp.bfloat16, lo, hi)
    def permutation(self, n):
        return jax.random.permutation(self._next(), n)


kernel_name = 'standalone__gqa_block_cached__near_ridge'

def setup_inputs():
    _rng = _Rng(jax.random.key(int.from_bytes(__import__("os").urandom(4), "little")))
    _w = (lambda a: (lambda t: t.astype(jnp.bfloat16) if jnp.issubdtype(t.dtype, jnp.floating) else t)(jnp.asarray(a)))
    B, Sq, D = 8, 96, 640
    Hq, Hkv, Sk, Dh = 32, 32, 512, 128
    assert Hq % Hkv == 0, (Hq, Hkv)
    return {
        "x": _w((lambda *s: _rng.normal(s) * 0.2)(B, Sq, D)),
        "k_cache": _w((lambda *s: _rng.normal(s) * 3.2)(B, Hkv, Sk, Dh)),
        "v_cache": _w((lambda *s: _rng.normal(s) * 0.05)(B, Hkv, Sk, Dh)),
        "wq": _w((lambda *s: _rng.normal(s) * 0.2)(D, Hq * Dh) * (D ** -0.5)),
        "wo": _w((lambda *s: _rng.normal(s) * 0.05)(Hq * Dh, D) * ((Hq * Dh) ** -0.5)),
    }

def reference(x, k_cache, v_cache, wq, wo):
    B, Sq, D = x.shape
    Hq, Dh = 32, 128
    Hkv = k_cache.shape[1]
    rep = Hq // Hkv
    q = (lambda x, *d: x.transpose(*d))((x @ wq).reshape(B, Sq, Hq, Dh), 0, 2, 1, 3)
    k = jnp.repeat(k_cache, rep, axis=1)
    v = jnp.repeat(v_cache, rep, axis=1)
    scores = jnp.einsum("bhqd,bhkd->bhqk", q, k) * (Dh ** -0.5)
    p = _softmax(scores, axis=-1)
    o = jnp.einsum("bhqk,bhkd->bhqd", p, v)
    return (lambda x, *d: x.transpose(*d))(o, 0, 2, 1, 3).reshape(B, Sq, Hq * Dh) @ wo
```

```python
import functools
import jax
import jax.numpy as jnp
import jax.experimental.pallas as pl
import jax.experimental.pallas.tpu as pltpu

HB = 8
NB = 3


def _kernel(x_hbm, k_hbm, v_hbm, wq_hbm, wo_hbm, o_hbm,
            xbuf, kbuf, vbuf, wqbuf, wobuf, acc_ref, obuf,
            x_sem, k_sem, v_sem, wq_sem, wo_sem, o_sem, *, hb, dh, nb, scale):
    g = pl.program_id(0)
    b = pl.program_id(1)
    ng = pl.num_programs(0)
    nbatch = pl.num_programs(1)
    step = g * nbatch + b
    nsteps = ng * nbatch
    w = hb * dh

    def kv_copies(s):
        gs = s // nbatch
        bs = s % nbatch
        slot = s % nb
        return (pltpu.make_async_copy(k_hbm.at[bs, pl.ds(gs * hb, hb)], kbuf.at[slot], k_sem.at[slot]),
                pltpu.make_async_copy(v_hbm.at[bs, pl.ds(gs * hb, hb)], vbuf.at[slot], v_sem.at[slot]))

    def wq_copy(gs):
        c = pl.multiple_of(gs * w, w)
        return pltpu.make_async_copy(wq_hbm.at[:, pl.ds(c, w)], wqbuf.at[:, pl.ds(c, w)], wq_sem.at[gs])

    def wo_copy(gs):
        c = pl.multiple_of(gs * w, w)
        return pltpu.make_async_copy(wo_hbm.at[pl.ds(c, w), :], wobuf.at[pl.ds(c, w), :], wo_sem.at[gs])

    def x_copy():
        return pltpu.make_async_copy(x_hbm, xbuf, x_sem.at[0])

    def o_copy(bs):
        return pltpu.make_async_copy(obuf.at[bs], o_hbm.at[bs], o_sem.at[bs])

    @pl.when(step == 0)
    def _():
        x_copy().start()
        wq_copy(0).start()
        for c in kv_copies(0):
            c.start()
        wo_copy(0).start()
        for s in range(1, nb - 1):
            for c in kv_copies(s):
                c.start()
        x_copy().wait()

    @pl.when(step + nb - 1 < nsteps)
    def _():
        for c in kv_copies(step + nb - 1):
            c.start()

    @pl.when(jnp.logical_and(b == 1, g + 1 < ng))
    def _():
        wq_copy(g + 1).start()
        wo_copy(g + 1).start()

    @pl.when(b == 0)
    def _():
        wq_copy(g).wait()

    slot = step % nb
    x = xbuf[b]

    @pl.when(b == 0)
    def _():
        wo_copy(g).wait()

    kc, vc = kv_copies(step)
    kc.wait()
    vc.wait()

    hh = hb // 2
    wh = hh * dh

    def qproj(j):
        c = pl.multiple_of(g * w + j * wh, wh)
        qq = jnp.dot(x, wqbuf[:, pl.ds(c, wh)], preferred_element_type=jnp.float32)
        return (qq * scale).astype(jnp.bfloat16)

    def oproj(j, outs):
        c = pl.multiple_of(g * w + j * wh, wh)
        return jnp.dot(jnp.concatenate(outs, axis=-1), wobuf[pl.ds(c, wh), :],
                       preferred_element_type=jnp.float32)

    qs = [qproj(0), None]

    def qk(h):
        qh = qs[h // hh][:, (h % hh) * dh:(h % hh + 1) * dh]
        return jax.lax.dot_general(qh, kbuf[slot, h], (((1,), (1,)), ((), ())),
                                   preferred_element_type=jnp.float32)
    outs = []
    s = qk(0)
    qs[1] = qproj(1)
    for h in range(hb):
        s_next = qk(h + 1) if h + 1 < hb else None
        if h == hb - 1:
            contrib = oproj(0, outs[:hh])
        m = jnp.max(s, axis=-1, keepdims=True)
        p = jnp.exp(s - m)
        l = jnp.sum(p, axis=-1, keepdims=True)
        o = jnp.dot(p.astype(jnp.bfloat16), vbuf[slot, h], preferred_element_type=jnp.float32)
        outs.append((o / l).astype(jnp.bfloat16))
        s = s_next
    contrib = contrib + oproj(1, outs[hh:])

    @pl.when(g == 0)
    def _():
        acc_ref[b] = contrib

    @pl.when(g > 0)
    def _():
        acc_ref[b] = acc_ref[b] + contrib

    @pl.when(g == ng - 1)
    def _():
        obuf[b] = acc_ref[b].astype(obuf.dtype)
        o_copy(b).start()

    @pl.when(step == nsteps - 1)
    def _():
        for bs in range(8):
            o_copy(bs).wait()


@jax.jit
def pallas_standalone__gqa_block_cached__near_ridge_kernel(x, k_cache, v_cache, wq, wo):
    B, Sq, D = x.shape
    _, Hkv, Sk, Dh = k_cache.shape
    Hq = wq.shape[1] // Dh
    assert Hq == Hkv
    hb = HB
    nb = NB
    ng = Hq // hb
    kern = functools.partial(_kernel, hb=hb, dh=Dh, nb=nb, scale=Dh ** -0.5)
    any_spec = pl.BlockSpec(memory_space=pl.ANY)
    return pl.pallas_call(
        kern,
        grid=(ng, B),
        in_specs=[any_spec] * 5,
        out_specs=any_spec,
        out_shape=jax.ShapeDtypeStruct((B, Sq, D), x.dtype),
        scratch_shapes=[
            pltpu.VMEM((B, Sq, D), x.dtype),
            pltpu.VMEM((nb, hb, Sk, Dh), k_cache.dtype),
            pltpu.VMEM((nb, hb, Sk, Dh), v_cache.dtype),
            pltpu.VMEM(wq.shape, wq.dtype),
            pltpu.VMEM(wo.shape, wo.dtype),
            pltpu.VMEM((B, Sq, D), jnp.float32),
            pltpu.VMEM((B, Sq, D), x.dtype),
            pltpu.SemaphoreType.DMA((1,)),
            pltpu.SemaphoreType.DMA((nb,)),
            pltpu.SemaphoreType.DMA((nb,)),
            pltpu.SemaphoreType.DMA((ng,)),
            pltpu.SemaphoreType.DMA((ng,)),
            pltpu.SemaphoreType.DMA((B,)),
        ],
        compiler_params=pltpu.CompilerParams(
            dimension_semantics=("arbitrary", "arbitrary"),
            vmem_limit_bytes=100 * 1024 * 1024),
    )(x, k_cache, v_cache, wq, wo)
```

```python
import functools
import jax
import jax.numpy as jnp
import jax.experimental.pallas as pl
import jax.experimental.pallas.tpu as pltpu

HB = 8
NB = 3
NSUB = 2


def _softmax_pv(s, v):
    m = jnp.max(s, axis=-1, keepdims=True)
    p = jnp.exp2(s - m)
    l = jnp.sum(p, axis=-1, keepdims=True)
    o = jnp.dot(p.astype(jnp.bfloat16), v, preferred_element_type=jnp.float32)
    return (o / l).astype(jnp.bfloat16)


def _kernel(x_hbm, k_hbm, v_hbm, wq_hbm, wo_hbm, o_hbm,
            xbuf, kbuf, vbuf, wqbuf, wobuf, qbuf, acc_ref, obuf,
            x_sem, k_sem, v_sem, ks_sem, vs_sem, wq_sem, wo_sem, o_sem, *, hb, dh, nb, nsub, scale):
    g = pl.program_id(0)
    b = pl.program_id(1)
    ng = pl.num_programs(0)
    nbatch = pl.num_programs(1)
    step = g * nbatch + b
    nsteps = ng * nbatch
    last = nsteps - 1
    w = hb * dh
    hs = hb // nsub

    def kv_copies(s):
        gs = s // nbatch
        bs = s % nbatch
        slot = s % nb
        return (pltpu.make_async_copy(k_hbm.at[bs, pl.ds(gs * hb, hb)], kbuf.at[slot], k_sem.at[slot]),
                pltpu.make_async_copy(v_hbm.at[bs, pl.ds(gs * hb, hb)], vbuf.at[slot], v_sem.at[slot]))

    def kv_sub_copies(j):
        gs = last // nbatch
        bs = last % nbatch
        slot = last % nb
        return (pltpu.make_async_copy(k_hbm.at[bs, pl.ds(gs * hb + j * hs, hs)],
                                      kbuf.at[slot, pl.ds(j * hs, hs)], ks_sem.at[j]),
                pltpu.make_async_copy(v_hbm.at[bs, pl.ds(gs * hb + j * hs, hs)],
                                      vbuf.at[slot, pl.ds(j * hs, hs)], vs_sem.at[j]))

    def wq_copy(gs):
        c = pl.multiple_of(gs * w, w)
        return pltpu.make_async_copy(wq_hbm.at[:, pl.ds(c, w)], wqbuf.at[:, pl.ds(c, w)], wq_sem.at[gs])

    def wo_copy(gs):
        c = pl.multiple_of(gs * w, w)
        return pltpu.make_async_copy(wo_hbm.at[pl.ds(c, w), :], wobuf.at[pl.ds(c, w), :], wo_sem.at[gs])

    def x_copy():
        return pltpu.make_async_copy(x_hbm, xbuf, x_sem.at[0])

    def o_copy(bs):
        return pltpu.make_async_copy(obuf.at[bs], o_hbm.at[bs], o_sem.at[bs])

    @pl.when(step == 0)
    def _():
        x_copy().start()
        wq_copy(0).start()
        for c in kv_copies(0):
            c.start()
        wq_copy(1).start()
        wo_copy(0).start()
        for s in range(1, nb - 1):
            for c in kv_copies(s):
                c.start()
        acc_ref[...] = jnp.zeros(acc_ref.shape, acc_ref.dtype)
        x_copy().wait()
        wq_copy(0).wait()

    @pl.when(step + nb - 1 < last)
    def _():
        for c in kv_copies(step + nb - 1):
            c.start()

    @pl.when(step + 2 == last)
    def _():
        for c in kv_sub_copies(0):
            c.start()

    @pl.when(step + 1 == last)
    def _():
        for c in kv_sub_copies(1):
            c.start()

    @pl.when(jnp.logical_and(b == 1, g + 2 < ng))
    def _():
        wq_copy(g + 2).start()

    @pl.when(jnp.logical_and(b == 4, g + 1 < ng))
    def _():
        wo_copy(g + 1).start()

    @pl.when(b == 0)
    def _():
        wo_copy(g).wait()

    @pl.when(jnp.logical_and(b == 0, g + 1 < ng))
    def _():
        wq_copy(g + 1).wait()

    slot = step % nb
    qslot = g % 2

    def qproj(gq):
        c = pl.multiple_of(gq * w, w)
        qq = jnp.dot(xbuf[b], wqbuf[:, pl.ds(c, w)], preferred_element_type=jnp.float32)
        return (qq * scale).astype(jnp.bfloat16)

    def oproj(c0, outs):
        c = pl.multiple_of(g * w + c0, dh)
        lhs = outs[0] if len(outs) == 1 else jnp.concatenate(outs, axis=-1)
        return jnp.dot(lhs, wobuf[pl.ds(c, len(outs) * dh), :], preferred_element_type=jnp.float32)

    def qk(h):
        qh = qbuf[qslot, b, :, h * dh:(h + 1) * dh]
        return jax.lax.dot_general(qh, kbuf[slot, h], (((1,), (1,)), ((), ())),
                                   preferred_element_type=jnp.float32)

    @pl.when(g == 0)
    def _():
        qbuf[0, b] = qproj(0)

    def body(next_q):
        kc, vc = kv_copies(step)
        kc.wait()
        vc.wait()
        hh = hb // 2
        wh = hh * dh
        outs = []
        s = qk(0)
        for h in range(hb):
            s_next = qk(h + 1) if h + 1 < hb else None
            if h == hb - 1:
                contrib = acc_ref[b] + oproj(0, outs[:hh])
                if next_q:
                    qbuf[1 - qslot, b] = qproj(g + 1)
            outs.append(_softmax_pv(s, vbuf[slot, h]))
            s = s_next
        contrib = contrib + oproj(wh, outs[hh:])
        acc_ref[b] = contrib
        if not next_q:
            obuf[b] = contrib.astype(obuf.dtype)
            o_copy(b).start()

    @pl.when(g < ng - 1)
    def _():
        body(True)

    @pl.when(jnp.logical_and(g == ng - 1, step < last))
    def _():
        body(False)

    @pl.when(step == last)
    def _():
        contrib = acc_ref[b]
        for j in range(nsub):
            kc, vc = kv_sub_copies(j)
            kc.wait()
            vc.wait()
            if j + 2 < nsub:
                for c in kv_sub_copies(j + 2):
                    c.start()
            outs = []
            h0 = j * hs
            s = qk(h0)
            for h in range(h0, h0 + hs):
                s_next = qk(h + 1) if h + 1 < h0 + hs else None
                outs.append(_softmax_pv(s, vbuf[slot, h]))
                s = s_next
            contrib = contrib + oproj(h0 * dh, outs)
        obuf[b] = contrib.astype(obuf.dtype)
        o_copy(b).start()
        for bs in range(o_sem.shape[0]):
            o_copy(bs).wait()


@jax.jit
def pallas_standalone__gqa_block_cached__near_ridge_kernel(x, k_cache, v_cache, wq, wo):
    B, Sq, D = x.shape
    _, Hkv, Sk, Dh = k_cache.shape
    Hq = wq.shape[1] // Dh
    assert Hq == Hkv
    hb = HB
    nb = NB
    nsub = NSUB
    ng = Hq // hb
    kern = functools.partial(_kernel, hb=hb, dh=Dh, nb=nb, nsub=nsub,
                             scale=Dh ** -0.5 * 1.4426950408889634)
    any_spec = pl.BlockSpec(memory_space=pl.ANY)
    return pl.pallas_call(
        kern,
        grid=(ng, B),
        in_specs=[any_spec] * 5,
        out_specs=any_spec,
        out_shape=jax.ShapeDtypeStruct((B, Sq, D), x.dtype),
        scratch_shapes=[
            pltpu.VMEM((B, Sq, D), x.dtype),
            pltpu.VMEM((nb, hb, Sk, Dh), k_cache.dtype),
            pltpu.VMEM((nb, hb, Sk, Dh), v_cache.dtype),
            pltpu.VMEM(wq.shape, wq.dtype),
            pltpu.VMEM(wo.shape, wo.dtype),
            pltpu.VMEM((2, B, Sq, hb * Dh), x.dtype),
            pltpu.VMEM((B, Sq, D), jnp.float32),
            pltpu.VMEM((B, Sq, D), x.dtype),
            pltpu.SemaphoreType.DMA((1,)),
            pltpu.SemaphoreType.DMA((nb,)),
            pltpu.SemaphoreType.DMA((nb,)),
            pltpu.SemaphoreType.DMA((nsub,)),
            pltpu.SemaphoreType.DMA((nsub,)),
            pltpu.SemaphoreType.DMA((ng,)),
            pltpu.SemaphoreType.DMA((ng,)),
            pltpu.SemaphoreType.DMA((B,)),
        ],
        compiler_params=pltpu.CompilerParams(
            dimension_semantics=("arbitrary", "arbitrary"),
            vmem_limit_bytes=100 * 1024 * 1024),
    )(x, k_cache, v_cache, wq, wo)
```

```python
import functools

import jax
import jax.numpy as jnp
import jax.experimental.pallas as pl
import jax.experimental.pallas.tpu as pltpu

HB = 8
NB = 3
NSUB = 2

_LOG2E = 1.4426950408889634


def _softmax_pv(s, v):
    m = jnp.max(s, axis=-1, keepdims=True)
    p = jnp.exp2(s - m)
    l = jnp.sum(p, axis=-1, keepdims=True)
    o = jnp.dot(p.astype(jnp.bfloat16), v, preferred_element_type=jnp.float32)
    return (o / l).astype(jnp.bfloat16)


def _kernel(x_hbm, k_hbm, v_hbm, wq_hbm, wo_hbm, o_hbm,
            xbuf, kbuf, vbuf, wqbuf, wobuf, qbuf, acc_ref, obuf,
            x_sem, k_sem, v_sem, ks_sem, vs_sem, wq_sem, wo_sem, o_sem,
            *, hb, dh, nb, nsub, scale):
    g = pl.program_id(0)
    b = pl.program_id(1)
    ng = pl.num_programs(0)
    nbatch = pl.num_programs(1)
    step = g * nbatch + b
    last = ng * nbatch - 1
    w = hb * dh
    hs = hb // nsub

    def kv_copies(s):
        gs = s // nbatch
        bs = s % nbatch
        slot = s % nb
        return (pltpu.make_async_copy(k_hbm.at[bs, pl.ds(gs * hb, hb)], kbuf.at[slot], k_sem.at[slot]),
                pltpu.make_async_copy(v_hbm.at[bs, pl.ds(gs * hb, hb)], vbuf.at[slot], v_sem.at[slot]))

    def kv_sub_copies(j):
        gs = last // nbatch
        bs = last % nbatch
        slot = last % nb
        return (pltpu.make_async_copy(k_hbm.at[bs, pl.ds(gs * hb + j * hs, hs)],
                                      kbuf.at[slot, pl.ds(j * hs, hs)], ks_sem.at[j]),
                pltpu.make_async_copy(v_hbm.at[bs, pl.ds(gs * hb + j * hs, hs)],
                                      vbuf.at[slot, pl.ds(j * hs, hs)], vs_sem.at[j]))

    def wq_copy(gs):
        c = pl.multiple_of(gs * w, w)
        return pltpu.make_async_copy(wq_hbm.at[:, pl.ds(c, w)], wqbuf.at[:, pl.ds(c, w)], wq_sem.at[gs])

    def wo_copy(gs):
        c = pl.multiple_of(gs * w, w)
        return pltpu.make_async_copy(wo_hbm.at[pl.ds(c, w), :], wobuf.at[pl.ds(c, w), :], wo_sem.at[gs])

    def x_copy():
        return pltpu.make_async_copy(x_hbm, xbuf, x_sem.at[0])

    def o_copy(bs):
        return pltpu.make_async_copy(obuf.at[bs], o_hbm.at[bs], o_sem.at[bs])

    @pl.when(step == 0)
    def _():
        x_copy().start()
        wq_copy(0).start()
        for c in kv_copies(0):
            c.start()
        wq_copy(1).start()
        wo_copy(0).start()
        for s in range(1, nb - 1):
            for c in kv_copies(s):
                c.start()
        acc_ref[...] = jnp.zeros(acc_ref.shape, acc_ref.dtype)
        x_copy().wait()
        wq_copy(0).wait()

    @pl.when(step + nb - 1 < last)
    def _():
        for c in kv_copies(step + nb - 1):
            c.start()

    @pl.when(step + 2 == last)
    def _():
        for c in kv_sub_copies(0):
            c.start()

    @pl.when(step + 1 == last)
    def _():
        for c in kv_sub_copies(1):
            c.start()

    @pl.when(jnp.logical_and(b == 1, g + 2 < ng))
    def _():
        wq_copy(g + 2).start()

    @pl.when(jnp.logical_and(b == 4, g + 1 < ng))
    def _():
        wo_copy(g + 1).start()

    @pl.when(b == 0)
    def _():
        wo_copy(g).wait()

    @pl.when(jnp.logical_and(b == 0, g + 1 < ng))
    def _():
        wq_copy(g + 1).wait()

    slot = step % nb
    qslot = g % 2

    def qproj(gq):
        c = pl.multiple_of(gq * w, w)
        qq = jnp.dot(xbuf[b], wqbuf[:, pl.ds(c, w)], preferred_element_type=jnp.float32)
        return (qq * scale).astype(jnp.bfloat16)

    def oproj(c0, outs):
        c = pl.multiple_of(g * w + c0, dh)
        lhs = outs[0] if len(outs) == 1 else jnp.concatenate(outs, axis=-1)
        return jnp.dot(lhs, wobuf[pl.ds(c, len(outs) * dh), :], preferred_element_type=jnp.float32)

    def qk(h):
        qh = qbuf[qslot, b, :, h * dh:(h + 1) * dh]
        return jax.lax.dot_general(qh, kbuf[slot, h], (((1,), (1,)), ((), ())),
                                   preferred_element_type=jnp.float32)

    @pl.when(g == 0)
    def _():
        qbuf[0, b] = qproj(0)

    def body(next_q):
        kc, vc = kv_copies(step)
        kc.wait()
        vc.wait()
        hh = hb // 2
        wh = hh * dh
        outs = []
        s = qk(0)
        for h in range(hb):
            s_next = qk(h + 1) if h + 1 < hb else None
            if h == hb - 1:
                contrib = acc_ref[b] + oproj(0, outs[:hh])
                if next_q:
                    qbuf[1 - qslot, b] = qproj(g + 1)
            outs.append(_softmax_pv(s, vbuf[slot, h]))
            s = s_next
        contrib = contrib + oproj(wh, outs[hh:])
        acc_ref[b] = contrib
        if not next_q:
            obuf[b] = contrib.astype(obuf.dtype)
            o_copy(b).start()

    @pl.when(g < ng - 1)
    def _():
        body(True)

    @pl.when(jnp.logical_and(g == ng - 1, step < last))
    def _():
        body(False)

    @pl.when(step == last)
    def _():
        contrib = acc_ref[b]
        for j in range(nsub):
            kc, vc = kv_sub_copies(j)
            kc.wait()
            vc.wait()
            if j + 2 < nsub:
                for c in kv_sub_copies(j + 2):
                    c.start()
            outs = []
            h0 = j * hs
            s = qk(h0)
            for h in range(h0, h0 + hs):
                s_next = qk(h + 1) if h + 1 < h0 + hs else None
                outs.append(_softmax_pv(s, vbuf[slot, h]))
                s = s_next
            contrib = contrib + oproj(h0 * dh, outs)
        obuf[b] = contrib.astype(obuf.dtype)
        o_copy(b).start()
        for bs in range(o_sem.shape[0]):
            o_copy(bs).wait()


@jax.jit
def pallas_standalone__gqa_block_cached__near_ridge_kernel(x, k_cache, v_cache, wq, wo):
    B, Sq, D = x.shape
    _, Hkv, Sk, Dh = k_cache.shape
    Hq = wq.shape[1] // Dh
    assert Hq == Hkv, "kernel is specialised to rep == 1 (Hq == Hkv)"
    hb, nb, nsub = HB, NB, NSUB
    ng = Hq // hb
    assert Hq % hb == 0 and ng >= 2 and B > 4 and nb >= 3 and nsub >= 2 and hb % (2 * nsub) == 0
    kern = functools.partial(_kernel, hb=hb, dh=Dh, nb=nb, nsub=nsub, scale=Dh ** -0.5 * _LOG2E)
    any_spec = pl.BlockSpec(memory_space=pl.ANY)
    return pl.pallas_call(
        kern,
        grid=(ng, B),
        in_specs=[any_spec] * 5,
        out_specs=any_spec,
        out_shape=jax.ShapeDtypeStruct((B, Sq, D), x.dtype),
        scratch_shapes=[
            pltpu.VMEM((B, Sq, D), x.dtype),
            pltpu.VMEM((nb, hb, Sk, Dh), k_cache.dtype),
            pltpu.VMEM((nb, hb, Sk, Dh), v_cache.dtype),
            pltpu.VMEM(wq.shape, wq.dtype),
            pltpu.VMEM(wo.shape, wo.dtype),
            pltpu.VMEM((2, B, Sq, hb * Dh), x.dtype),
            pltpu.VMEM((B, Sq, D), jnp.float32),
            pltpu.VMEM((B, Sq, D), x.dtype),
            pltpu.SemaphoreType.DMA((1,)),
            pltpu.SemaphoreType.DMA((nb,)),
            pltpu.SemaphoreType.DMA((nb,)),
            pltpu.SemaphoreType.DMA((nsub,)),
            pltpu.SemaphoreType.DMA((nsub,)),
            pltpu.SemaphoreType.DMA((ng,)),
            pltpu.SemaphoreType.DMA((ng,)),
            pltpu.SemaphoreType.DMA((B,)),
        ],
        compiler_params=pltpu.CompilerParams(
            dimension_semantics=("arbitrary", "arbitrary"),
            vmem_limit_bytes=64 * 1024 * 1024),
    )(x, k_cache, v_cache, wq, wo)
```
